```python
import os as _os
_os.environ.setdefault("JAX_PLATFORMS", "cpu")
import jax
import jax.numpy as jnp

def _softmax(x, axis=-1):
    return jax.nn.softmax(x, axis=axis)
def _gelu(x):
    return jax.nn.gelu(x, approximate=True)
def _silu(x):
    return jax.nn.silu(x)
def _sigmoid(x):
    return jax.nn.sigmoid(x)
def _layernorm(x, axis=-1, eps=1e-5):
    m = jnp.mean(x, axis=axis, keepdims=True)
    v = jnp.var(x, axis=axis, keepdims=True)
    return (x - m) / jnp.sqrt(v + eps)
def _scatter_add(tgt, idx, src, axis=0):
    return tgt.at[idx].add(src)
def _segment_sum(src, seg, n):
    return jax.ops.segment_sum(src, seg, n)
class _Rng:
    def __init__(self, key):
        self._k = key
    def _next(self):
        self._k, sub = jax.random.split(self._k)
        return sub
    def normal(self, shape):
        return jax.random.normal(self._next(), shape, dtype=jnp.bfloat16)
    def randint(self, lo, hi, shape):
        return jax.random.randint(self._next(), shape, lo, hi, dtype=jnp.int32)
    def uniform(self, shape, lo=0.0, hi=1.0):
        return jax.random.uniform(self._next(), shape, jnp.bfloat16, lo, hi)
    def permutation(self, n):
        return jax.random.permutation(self._next(), n)


kernel_name = 'concat_heads__gqa_block_cached__mha_block_cached__near_ridge'

def setup_inputs():
    _rng = _Rng(jax.random.key(int.from_bytes(__import__("os").urandom(4), "little")))
    _w = (lambda a: (lambda t: t.astype(jnp.bfloat16) if jnp.issubdtype(t.dtype, jnp.floating) else t)(jnp.asarray(a)))
    def _A_setup():
        B, Sq, D = 8, 112, 448
        Hq, Hkv, Sk, Dh = 16, 8, 512, 256
        assert Hq % Hkv == 0, (Hq, Hkv)
        return {
            "x": _w((lambda *s: _rng.normal(s) * 0.8)(B, Sq, D)),
            "k_cache": _w((lambda *s: _rng.normal(s) * 0.8)(B, Hkv, Sk, Dh)),
            "v_cache": _w((lambda *s: _rng.normal(s) * 0.05)(B, Hkv, Sk, Dh)),
            "wq": _w((lambda *s: _rng.normal(s) * 0.8)(D, Hq * Dh) * (D ** -0.5)),
            "wo": _w((lambda *s: _rng.normal(s) * 0.05)(Hq * Dh, D) * ((Hq * Dh) ** -0.5)),
        }
    _A_in = _A_setup()

    def _B_setup():
        B, Sq, D = 8, 112, 448
        H, Sk, Dh = 16, 512, 256
        return {
            "x": _w((lambda *s: _rng.normal(s) * 0.8)(B, Sq, D)),
            "k_cache": _w((lambda *s: _rng.normal(s) * 0.8)(B, H, Sk, Dh)),
            "v_cache": _w((lambda *s: _rng.normal(s) * 0.05)(B, H, Sk, Dh)),
            "wq": _w((lambda *s: _rng.normal(s) * 0.8)(D, H * Dh) * (D ** -0.5)),
            "wo": _w((lambda *s: _rng.normal(s) * 0.05)(H * Dh, D) * ((H * Dh) ** -0.5)),
        }
    _B_in = _B_setup()

    return {
        "A_x": _A_in["x"],
        "A_k_cache": _A_in["k_cache"],
        "A_v_cache": _A_in["v_cache"],
        "A_wq": _A_in["wq"],
        "A_wo": _A_in["wo"],
        "B_x": _B_in["x"],
        "B_k_cache": _B_in["k_cache"],
        "B_v_cache": _B_in["v_cache"],
        "B_wq": _B_in["wq"],
        "B_wo": _B_in["wo"],
    }

def reference(A_x, A_k_cache, A_v_cache, A_wq, A_wo, B_x, B_k_cache, B_v_cache, B_wq, B_wo):
    def _A_ref(x, k_cache, v_cache, wq, wo):
        B, Sq, D = x.shape
        Hq, Dh = 16, 256
        Hkv = k_cache.shape[1]
        rep = Hq // Hkv
        q = (lambda x, *d: x.transpose(*d))((x @ wq).reshape(B, Sq, Hq, Dh), 0, 2, 1, 3)
        k = jnp.repeat(k_cache, rep, axis=1)
        v = jnp.repeat(v_cache, rep, axis=1)
        scores = jnp.einsum("bhqd,bhkd->bhqk", q, k) * (Dh ** -0.5)
        p = _softmax(scores, axis=-1)
        o = jnp.einsum("bhqk,bhkd->bhqd", p, v)
        return (lambda x, *d: x.transpose(*d))(o, 0, 2, 1, 3).reshape(B, Sq, Hq * Dh) @ wo

    def _B_ref(x, k_cache, v_cache, wq, wo):
        B, Sq, D = x.shape
        H, Dh = 16, 256
        q = (lambda x, *d: x.transpose(*d))((x @ wq).reshape(B, Sq, H, Dh), 0, 2, 1, 3)
        scores = jnp.einsum("bhqd,bhkd->bhqk", q, k_cache) * (Dh ** -0.5)
        p = _softmax(scores, axis=-1)
        o = jnp.einsum("bhqk,bhkd->bhqd", p, v_cache)
        return (lambda x, *d: x.transpose(*d))(o, 0, 2, 1, 3).reshape(B, Sq, H * Dh) @ wo

    a = _A_ref(A_x, A_k_cache, A_v_cache, A_wq, A_wo)
    b = _B_ref(B_x, B_k_cache, B_v_cache, B_wq, B_wo)
    return jnp.concatenate([a, b], axis=-1)
```

```python
import numpy as np
import jax
import jax.numpy as jnp
from jax import lax
import jax.experimental.pallas as pl
import jax.experimental.pallas.tpu as pltpu

F32, BF16 = jnp.float32, jnp.bfloat16
NT = (((1,), (1,)), ((), ()))
NB, SQ, D, SK, DH = 8, 112, 448, 512, 256
T = NB * SQ
NG = 8
NTILE = T // 128
RING = 16


def _mult(i, n, align=None):
    return i * n if isinstance(i, int) else pl.multiple_of(i * n, align or n)


def program(order):
    ops = []
    if order == 0:
        fill = [[], []] + [[("op", t, 0)] for t in range(5)] + [[("op", 5, 0)]]
        last = [("op", 6, 0)]
    else:
        fill = [[("op", 5, 1)], [("op", 6, 1)]] + [[("op", t, 0)] for t in range(5)] + [[]]
        last = []
    if order == 4:
        fill = [[("op", 6, 1)], []] + [[("op", t, 0)] for t in range(6)]
    if order == 5:
        fill = [[], [("op", 6, 1)]] + [[("op", t, 0)] for t in range(6)]
    if order in (0, 1, 4, 5):
        for b in range(NB):
            ops += [("qk", b, 0), ("qk", b, 1)] + fill[b] + [("pv", b, 0), ("pv", b, 1)]
    elif order == 2:
        for b in range(NB - 2):
            ops += [("qk", b, 0), ("qk", b, 1)] + fill[b] + [("pv", b, 0), ("pv", b, 1)]
        ops += [("qk", 6, 0), ("qk", 6, 1), ("qk", 7, 0), ("pv", 6, 0), ("qk", 7, 1), ("pv", 6, 1),
                ("op", 4, 0), ("pv", 7, 0), ("pv", 7, 1)]
    elif order == 3:
        heads = [(b, j) for b in range(NB) for j in range(2)]
        fl = {0: ("op", 5, 1), 2: ("op", 6, 1), 5: ("op", 0, 0), 7: ("op", 1, 0), 9: ("op", 2, 0),
              11: ("op", 3, 0), 14: ("op", 4, 0)}
        ops += [("qk",) + heads[0], ("qk",) + heads[1]]
        for i in range(16):
            if i in fl:
                ops.append(fl[i])
            ops.append(("pv",) + heads[i])
            if i + 2 < 16:
                ops.append(("qk",) + heads[i + 2])
    return ops + last


def build(order=4, torder=4, gpi=1, qpn=2, qp1=2, nfine=2, nob=True, tcuts=(0, 4, 6), nodma=0, nocomp=0, flags=None, prof=0, xsplit=1, wqcuts=(1, 2, 4, 8)):
    scale = float(DH ** -0.5 * np.log2(np.e))
    tcuts = tuple(tcuts) + (NB,)

    def body(ax, ak, av, awq, awo, bx, bk, bv, bwq, bwo, out,
             xbuf, wqbuf, wobuf, kbuf, vbuf, qo, acc, obuf,
             qsem, gsem, osem):
        def x_copy(p):
            return [pltpu.make_async_copy((ax, bx)[p], xbuf.at[p], qsem.at[qstep(p * NG)])]

        def w_copy(src, dst, p, g, sem):
            return [pltpu.make_async_copy(src[p].at[:, pl.ds(_mult(g, 512), 512)], dst.at[p * NG + g], sem)]

        def qstep(i):
            return jnp.where(i < qp1, i, qp1 + (i - qp1) // qpn) if qp1 else i // qpn

        def wq_copy(p, g):
            return w_copy((awq, bwq), wqbuf, p, g, qsem.at[qstep(p * NG + g)])

        def b_slot(g):
            return (8 + 2 * g) % RING if isinstance(g, int) else lax.rem(8 + 2 * g, RING)

        def group_copy(p, g):
            src = pl.ds((p + 1) * g, p + 1)
            dst = pl.ds(b_slot(g) if p else g, p + 1)
            return [pltpu.make_async_copy((ak, bk)[p].at[:, src], kbuf.at[:, dst], gsem.at[g]),
                    pltpu.make_async_copy((av, bv)[p].at[:, src], vbuf.at[:, dst], gsem.at[g])
                    ] + w_copy((awo, bwo), wobuf, p, g, gsem.at[g])

        def tail_copy(g, n):
            bs = pl.ds(tcuts[n], tcuts[n + 1] - tcuts[n])
            src, dst = pl.ds(2 * g, 2), pl.ds(b_slot(g), 2)
            sem = qsem.at[(g - NG + nfine) * (len(tcuts) - 1) + n]
            return [pltpu.make_async_copy(bk.at[bs, src], kbuf.at[bs, dst], sem),
                    pltpu.make_async_copy(bv.at[bs, src], vbuf.at[bs, dst], sem)
                    ] + (w_copy((awo, bwo), wobuf, 1, g, sem) if n == 0 else [])

        def out_copy(t):
            return [pltpu.make_async_copy(obuf.at[t], out.at[pl.ds(_mult(t, 128), 128)], osem)]

        def start(cs):
            for c in cs:
                if not nodma:
                    c.start()

        def wait(cs):
            if prof:
                with jax.named_scope("wait"):
                    for c in cs:
                        c.wait()
                return
            for c in cs:
                if not nodma:
                    c.wait()

        def qproj(i):
            if nocomp:
                return
            q = jnp.dot(xbuf[i // NG], wqbuf[i], preferred_element_type=F32) * scale
            q = q.astype(BF16)
            for c in range(4):
                qo[i * 4 + c] = q[:, c * 128:(c + 1) * 128]

        def qk(i, b, j, slot):
            rows, kt = pl.ds(_mult(b, SQ, 16), SQ), i * 4 + 2 * j
            q = jnp.concatenate([qo[kt, rows, :], qo[kt + 1, rows, :]], axis=1)
            return lax.dot_general(q, kbuf[b, slot], NT, preferred_element_type=F32)

        def pv(i, b, j, slot, s):
            rows, kt = pl.ds(_mult(b, SQ, 16), SQ), i * 4 + 2 * j
            m = jnp.max(s, axis=-1, keepdims=True)
            e = jnp.exp2(s - m)
            inv = 1.0 / jnp.sum(e, axis=-1, keepdims=True)
            o = (jnp.dot(e.astype(BF16), vbuf[b, slot], preferred_element_type=F32) * inv).astype(BF16)
            for c in range(2):
                qo[kt + c, rows, :] = o[:, c * 128:(c + 1) * 128]

        def oproj(i, t, tacc=None):
            trows = pl.ds(_mult(t, 128), 128)
            o = jnp.concatenate([qo[i * 4 + c, trows, :] for c in range(4)], axis=1)
            r = lax.dot_general(wobuf[i], o, NT, preferred_element_type=F32)
            acc[i // NG, t if tacc is None else tacc] += r

        def finish(t):
            for c in range(NTILE):
                lo, hi = c * 128, (c + 1) * 128
                parts = ([acc[0, t, lo:min(hi, D), :]] if lo < D else []) + \
                        ([acc[1, t, max(lo, D) - D:hi - D, :]] if hi > D else [])
                obuf[t, :, lo:hi] = jnp.concatenate(parts, axis=0).T.astype(BF16)

        start(x_copy(0) + wq_copy(0, 0))

        def issue_w(i, c):
            pl.when(i < NG)(lambda: start(wq_copy(0, i)))
            pl.when(i == NG)(lambda: start(x_copy(1)))
            pl.when(i >= NG)(lambda: start(wq_copy(1, i - NG)))
            return c
        lax.fori_loop(1, 2 * NG, issue_w, 0)

        def issue_a(g, c):
            start(group_copy(0, g))
            return c
        lax.fori_loop(0, NG, issue_a, 0)
        acc[...] = jnp.zeros(acc.shape, F32)

        def issue_b(g):
            pl.when(g < NG - nfine)(lambda: start(group_copy(1, g)))

            @pl.when(g >= NG - nfine)
            def _():
                def one(n, c):
                    for m in range(len(tcuts) - 1):
                        pl.when(n == m)(lambda m=m: start(tail_copy(g, m)))
                    return c
                lax.fori_loop(0, len(tcuts) - 1, one, 0)

        def step_q(i, n):
            pl.when(i == 0)(lambda: wait(x_copy(0)))
            pl.when(i == NG)(lambda: wait(x_copy(1)))
            for d in range(n):
                pl.when(i < NG)(lambda: wait(wq_copy(0, i + d)))
                pl.when(i >= NG)(lambda: wait(wq_copy(1, i + d - NG)))
            for d in range(n):
                qproj(i + d)
        if qp1:
            lax.fori_loop(0, qp1, lambda n, c: step_q(n, 1), None)
        lax.fori_loop(0, (2 * NG - qp1) // qpn, lambda n, c: step_q(qp1 + n * qpn, qpn), None)

        def run(i, slots, order, waits=None, last=None, first=True):
            prev, s, done = jnp.maximum(i - 1, 0), {}, []
            for op, a, j in program(order):
                if op == "qk" and j == 0 and waits and a in waits:
                    wait(waits.pop(a))
                if done and not waits:
                    pl.when(last)(lambda: start(sum((out_copy(t) for t in done), [])))
                    done.clear()
                if nocomp:
                    continue
                if op == "qk":
                    s[a, j] = qk(i, a, j, slots[j])
                elif op == "pv":
                    pv(i, a, j, slots[j], s.pop((a, j)))
                elif j:
                    oproj(prev, a, jnp.where(i == 0, NTILE, a) if first else None)
                else:
                    oproj(i, a)
                    if last is not None:
                        finish(a)
                        done.append(a)

        def step(n, c):
            for i in (n * gpi + d for d in range(gpi)):
                pl.when(i < NG)(lambda: wait(group_copy(0, i)))
                pl.when(i >= NG)(lambda: wait(group_copy(1, i - NG)))
                pl.when(i < 4)(lambda: issue_b(i))
                pl.when(jnp.logical_and(i >= 6, i < NG + 2))(lambda: issue_b(i - 2))
            for d in range(gpi):
                i = n * gpi + d
                run(i, [jnp.where(i < NG, i, lax.rem(2 * i - NG + j, RING)) for j in range(2)], order, first=d == 0)
            return c
        lax.fori_loop(0, (2 * NG - nfine) // gpi, step, 0)

        def step_tail(g, c):
            run(NG + g, [b_slot(g), b_slot(g) + 1], torder,
                {b: tail_copy(g, n) for n, b in enumerate(tcuts[:-1])}, g == NG - 1, False)
            return c
        lax.fori_loop(NG - nfine, NG, step_tail, 0)
        if nocomp:
            start(sum((out_copy(t) for t in range(NTILE)), []))
        else:
            oproj(2 * NG - 1, NTILE - 1)
            finish(NTILE - 1)
            start(out_copy(NTILE - 1))
        wait(sum((out_copy(t) for t in range(NTILE)), []))

    def f(ax, ak, av, awq, awo, bx, bk, bv, bwq, bwo):
        hbm = pl.BlockSpec(memory_space=pl.ANY)
        out = pl.pallas_call(
            body,
            out_shape=jax.ShapeDtypeStruct((T, 2 * D), BF16),
            in_specs=[hbm] * 10,
            out_specs=hbm,
            scratch_shapes=[
                pltpu.VMEM((2, T, D), BF16),
                pltpu.VMEM((2 * NG, D, 512), BF16),
                pltpu.VMEM((2 * NG, D, 512), BF16),
                pltpu.VMEM((NB, RING, SK, DH), BF16),
                pltpu.VMEM((NB, RING, SK, DH), BF16),
                pltpu.VMEM((8 * NG, T, 128), BF16),
                pltpu.VMEM((2, NTILE + 1, D, 128), F32),
                pltpu.VMEM((NTILE, 128, 2 * D), BF16),
                pltpu.SemaphoreType.DMA((max(qp1 + (2 * NG - qp1) // qpn, nfine * (len(tcuts) - 1)),)),
                pltpu.SemaphoreType.DMA((NG,)),
                pltpu.SemaphoreType.DMA(()),
            ],
            compiler_params=pltpu.CompilerParams(vmem_limit_bytes=120 * 2**20, flags=flags,
                                                 disable_bounds_checks=nob),
        )(ax.reshape(T, D), ak, av, awq, awo.T, bx.reshape(T, D), bk, bv, bwq, bwo.T)
        return out.reshape(NB, SQ, 2 * D)
    return f


@jax.jit
def pallas_concat_heads__gqa_block_cached__mha_block_cached__near_ridge_kernel(
        A_x, A_k_cache, A_v_cache, A_wq, A_wo, B_x, B_k_cache, B_v_cache, B_wq, B_wo):
    return build(tcuts=(0, 3, 6))(A_x, A_k_cache, A_v_cache, A_wq, A_wo, B_x, B_k_cache, B_v_cache, B_wq, B_wo)
```

```python
import numpy as np
import jax
import jax.numpy as jnp
from jax import lax
import jax.experimental.pallas as pl
import jax.experimental.pallas.tpu as pltpu

F32, BF16 = jnp.float32, jnp.bfloat16
NT = (((1,), (1,)), ((), ()))

NB, SQ, D, SK, DH = 8, 112, 448, 512, 256
T = NB * SQ
NG = 8
GW = 2 * DH
NTILE = T // 128
RING = 16
NX = 4
QPN = 3
NQSTEP = (2 * NG - 1) // QPN
NPAIR = 6
CUTS = (0, 4, 6, NB)
NCUT = len(CUTS) - 1
KV_ROWS = 64
W_ROWS = 32
BULK, TRICKLE = 1, 0
SCALE = float(DH ** -0.5 * np.log2(np.e))


def _mult(i, n, align=None):
    return i * n if isinstance(i, int) else pl.multiple_of(i * n, align or n)


def _start(copies, priority=BULK):
    for c in copies:
        c.start(priority=priority)


def _wait(copies):
    for c in copies:
        c.wait()


def _body(ax, ak, av, awq, awo_t, bx, bk, bv, bwq, bwo_t, out,
          xbuf, wbuf, kvbuf, qo, acc, obuf, xsem, qsem, wsem, kvsem, osem):

    def xa_copy(r):
        rows = pl.ds(_mult(r, T // NX, 16), T // NX)
        return [pltpu.make_async_copy(ax.at[rows], xbuf.at[0, rows], xsem.at[r])]

    def xb_copy():
        return [pltpu.make_async_copy(bx, xbuf.at[1], xsem.at[NX])]

    def w_copy(k, g, sem, rows=slice(None)):
        src = (awq, bwq, awo_t, bwo_t)[k]
        return [pltpu.make_async_copy(src.at[rows, pl.ds(_mult(g, GW), GW)], wbuf.at[k * NG + g, rows], sem)]

    def wq_copy(p, g):
        return w_copy(p, g, qsem.at[(p * NG + g - 1) // QPN])

    def wo_copy(p, g, rows=slice(None)):
        return w_copy(2 + p, g, wsem.at[p * NG + g], rows)

    def b_slot(g):
        return (NG + 2 * g) & (RING - 1)

    def kv_copy(p, bs, src, dst, s, rows=slice(None)):
        return [pltpu.make_async_copy(cache.at[bs, src, rows], kvbuf.at[which, bs, dst, rows], kvsem.at[s])
                for which, cache in enumerate(((ak, av), (bk, bv))[p])]

    def kv_total(bs, dst, s):
        part = kvbuf.at[:, bs, dst]
        return [pltpu.make_async_copy(part, part, kvsem.at[s])]

    def group_wait(p, g):
        _wait(kv_total(slice(None), pl.ds(b_slot(g) if p else g, p + 1), p * NG + g) + wo_copy(p, g))

    def tail_sem(g, n):
        return NG + g if n == 0 else 2 * NG + (g - NG + 2) * (NCUT - 1) + n - 1

    def out_copy(t, c0=0, c1=NTILE):
        cols = pl.ds(c0 * 128, (c1 - c0) * 128)
        return [pltpu.make_async_copy(obuf.at[t, :, cols], out.at[pl.ds(t * 128, 128), cols], osem)]

    def trickle_wo(half, m, p):
        rows = pl.ds(pl.multiple_of((half & 1) * (D // 2) + m * W_ROWS, W_ROWS), W_ROWS)
        _start(wo_copy(p, half >> 1, rows), TRICKLE)

    def trickle_kv(i, m, which):
        g = (i >> 1) + (i >= 2 * (NG - 2)).astype(jnp.int32)
        j, r = divmod(m, SK // KV_ROWS)
        copies = kv_copy(1, i & 1, 2 * g + j, b_slot(g) + j, NG + g, pl.ds(r * KV_ROWS, KV_ROWS))
        _start(copies[which:which + 1], TRICKLE)

    def qproj(i, r0, n, c0, nc):
        q = jnp.dot(xbuf[i // NG, pl.ds(r0, n)], wbuf[i, :, c0 * 128:(c0 + nc) * 128],
                    preferred_element_type=F32)
        q = (q * SCALE).astype(BF16)
        for c in range(nc):
            qo[i * 4 + c0 + c, pl.ds(r0, n), :] = q[:, c * 128:(c + 1) * 128]

    def load_qo(kt, n, rows):
        return jnp.concatenate([qo[kt + c, rows, :] for c in range(n)], axis=1)

    def scores(i, b, j, slot):
        q = load_qo(i * 4 + 2 * j, 2, pl.ds(b * SQ, SQ))
        return lax.dot_general(q, kvbuf[0, b, slot], NT, preferred_element_type=F32)

    def attend(i, b, j, slot, s):
        e = jnp.exp2(s - jnp.max(s, axis=-1, keepdims=True))
        l = jnp.sum(e, axis=-1, keepdims=True)
        inv = pl.reciprocal(l, approx=True)
        inv = inv * (2.0 - l * inv)
        o = (jnp.dot(e.astype(BF16), kvbuf[1, b, slot], preferred_element_type=F32) * inv).astype(BF16)
        for c in range(2):
            qo[i * 4 + 2 * j + c, pl.ds(b * SQ, SQ), :] = o[:, c * 128:(c + 1) * 128]

    def oproj(i, t, t_acc):
        o = load_qo(i * 4, 4, pl.ds(t * 128, 128))
        acc[i // NG, t_acc] += lax.dot_general(wbuf[2 * NG + i], o, NT, preferred_element_type=F32)

    def finish(t, c0=0, c1=NTILE):
        for c in range(c0, c1):
            lo, hi = c * 128, (c + 1) * 128
            parts = ([acc[0, t, lo:min(hi, D), :]] if lo < D else []) + \
                    ([acc[1, t, max(lo, D) - D:hi - D, :]] if hi > D else [])
            obuf[t, :, lo:hi] = jnp.concatenate(parts, axis=0).T.astype(BF16)

    def group(i, slots, first=False, last=None):
        done = []

        def flush(b):
            if done and b >= CUTS[-2]:
                copies = sum((out_copy(t) for t in done), [])
                pl.when(last)(lambda: _start(copies))
                done.clear()

        for b in range(NB):
            if last is not None and b in CUTS:
                n = CUTS.index(b)
                _wait(kv_total(pl.ds(b, CUTS[n + 1] - b), pl.ds(slots[0], 2), tail_sem(i - NG, n)))
                flush(b)
            s = []
            for j in range(2):
                s.append(scores(i, b, j, slots[j]))
                if last is None:
                    trickle_kv(i, 2 * b + j, 0)
            if b == 0 and first:
                oproj(jnp.maximum(i - 1, 0), NTILE - 1, jnp.where(i == 0, NTILE, NTILE - 1))
            elif b == 0:
                oproj(i - 1, NTILE - 1, NTILE - 1)
            elif b >= 2:
                oproj(i, b - 2, b - 2)
                if last is not None:
                    finish(b - 2)
                    done.append(b - 2)
                    flush(b)
            for j in range(2):
                attend(i, b, j, slots[j], s[j])
                if last is None:
                    trickle_kv(i, 2 * b + j, 1)

    first_wq = w_copy(0, 0, xsem.at[NX + 1])
    _start(xa_copy(0) + first_wq)
    lax.fori_loop(1, NX, lambda r, c: _start(xa_copy(r)), None)
    lax.fori_loop(1, NG, lambda g, c: _start(wq_copy(0, g)), None)
    _start(xb_copy())
    lax.fori_loop(0, NG, lambda g, c: _start(wq_copy(1, g)), None)
    for p in range(2):
        _start(wo_copy(p, NG - 1, pl.ds(D // 2, D // 2)))
    lax.fori_loop(0, NG, lambda g, c: _start(kv_copy(0, slice(None), g, g, g)), None)
    acc[...] = jnp.zeros(acc.shape, F32)

    def first_q_step(r, carry):
        pl.when(r == 0)(lambda: _wait(first_wq))
        _wait(xa_copy(r))
        qproj(0, _mult(r, T // NX, 16), T // NX, 0, 4)
    lax.fori_loop(0, NX, first_q_step, None)

    def q_step(n, carry):
        pl.when(n == (NG - 1) // QPN)(lambda: _wait(xb_copy()))
        chunks = wbuf.at[pl.ds(1 + n * QPN, QPN)]
        pltpu.make_async_copy(chunks, chunks, qsem.at[n]).wait()
        for d in range(QPN):
            i = 1 + n * QPN + d
            for m in range(NTILE):
                for p in range(2):
                    qproj(i, m * 128, 128, 2 * p, 2)
                    trickle_wo(i - 1, m, p)
    lax.fori_loop(0, NQSTEP, q_step, None)

    def issue_b(g):
        _start(kv_copy(1, pl.ds(2, NB - 2), pl.ds(2 * g, 2), pl.ds(b_slot(g), 2), NG + g))

    def issue_tail():
        for g, b0 in ((NG - 2, 0), (NG - 1, 2)):
            for n in range(NCUT):
                lo = max(CUTS[n], b0)
                _start(kv_copy(1, pl.ds(lo, CUTS[n + 1] - lo), pl.ds(2 * g, 2), pl.ds(b_slot(g), 2), tail_sem(g, n)))

    def pair_step(n, carry):
        for i in (2 * n, 2 * n + 1):
            pl.when(i < NG)(lambda: group_wait(0, i))
            pl.when(i >= NG)(lambda: group_wait(1, i - NG))
            pl.when(i < 4)(lambda: issue_b(i))
            pl.when((i >= 6) & (i < NG))(lambda: issue_b(i - 2))
        pl.when(2 * n == NG)(issue_tail)
        for i, first in ((2 * n, True), (2 * n + 1, False)):
            group(i, [jnp.where(i < NG, i, b_slot(i - NG) + j) for j in range(2)], first)
    lax.fori_loop(0, NPAIR, pair_step, None)

    def single_step(g, carry):
        group_wait(1, g)
        group(NG + g, [b_slot(g), b_slot(g) + 1])
    lax.fori_loop(2 * NPAIR - NG, NG - 2, single_step, None)

    def tail_step(g, carry):
        _wait(wo_copy(1, g))
        group(NG + g, [b_slot(g), b_slot(g) + 1], last=g == NG - 1)
    lax.fori_loop(NG - 2, NG, tail_step, None)

    t = NTILE - 1
    finish(t, 0, 3)
    _start(out_copy(t, 0, 3))
    oproj(2 * NG - 1, t, t)
    finish(t, 3, NTILE)
    _start(out_copy(t, 3, NTILE))
    _wait(sum((out_copy(u) for u in range(t)), []) + out_copy(t, 0, 3) + out_copy(t, 3, NTILE))


@jax.jit
def pallas_concat_heads__gqa_block_cached__mha_block_cached__near_ridge_kernel(
    A_x: jax.Array,
    A_k_cache: jax.Array,
    A_v_cache: jax.Array,
    A_wq: jax.Array,
    A_wo: jax.Array,
    B_x: jax.Array,
    B_k_cache: jax.Array,
    B_v_cache: jax.Array,
    B_wq: jax.Array,
    B_wo: jax.Array,
):
    hbm = pl.BlockSpec(memory_space=pl.ANY)
    out = pl.pallas_call(
        _body,
        out_shape=jax.ShapeDtypeStruct((T, 2 * D), BF16),
        in_specs=[hbm] * 10,
        out_specs=hbm,
        scratch_shapes=[
            pltpu.VMEM((2, T, D), BF16),
            pltpu.VMEM((4 * NG, D, GW), BF16),
            pltpu.VMEM((2, NB, RING, SK, DH), BF16),
            pltpu.VMEM((8 * NG, T, 128), BF16),
            pltpu.VMEM((2, NTILE + 1, D, 128), F32),
            pltpu.VMEM((NTILE, 128, 2 * D), BF16),
            pltpu.SemaphoreType.DMA((NX + 2,)),
            pltpu.SemaphoreType.DMA((NQSTEP,)),
            pltpu.SemaphoreType.DMA((2 * NG,)),
            pltpu.SemaphoreType.DMA((2 * NG + 2 * (NCUT - 1),)),
            pltpu.SemaphoreType.DMA(()),
        ],
        compiler_params=pltpu.CompilerParams(vmem_limit_bytes=120 * 2**20, disable_semaphore_checks=True),
    )(A_x.reshape(T, D), A_k_cache, A_v_cache, A_wq, A_wo.T,
      B_x.reshape(T, D), B_k_cache, B_v_cache, B_wq, B_wo.T)
    return out.reshape(NB, SQ, 2 * D)
```

```python
import numpy as np
import jax
import jax.numpy as jnp
from jax import lax
import jax.experimental.pallas as pl
import jax.experimental.pallas.tpu as pltpu

F32, BF16 = jnp.float32, jnp.bfloat16
NT = (((1,), (1,)), ((), ()))

NB, SQ, D, SK, DH = 8, 112, 448, 512, 256
T = NB * SQ
NG = 8
GW = 2 * DH
NTILE = T // 128
RING = 16
XCUTS = (0, 128, 384, T)
NX = len(XCUTS) - 1
QPN = 3
NQSTEP = (2 * NG - 1) // QPN
NPAIR = 6
CUTS = (0, 4, 6, NB)
NCUT = len(CUTS) - 1
KV_ROWS = 64
TRICKLED = (2, 2, 2, 3, 1, 2, 0, 2)
BULK, TRICKLE = 1, 0
SCALE = float(DH ** -0.5 * np.log2(np.e))


def _mult(i, n):
    return i * n if isinstance(i, int) else pl.multiple_of(i * n, n)


def _start(copies, priority=BULK):
    for c in copies:
        c.start(priority=priority)


def _wait(copies):
    for c in copies:
        c.wait()


def _body(ax, ak, av, awq, awo_t, bx, bk, bv, bwq, bwo_t, out,
          xbuf, wbuf, kvbuf, qo, acc, obuf, xsem, qsem, wsem, kvsem, osem):

    def xa_copy(r):
        rows = pl.ds(XCUTS[r], XCUTS[r + 1] - XCUTS[r])
        return [pltpu.make_async_copy(ax.at[rows], xbuf.at[0, rows], xsem.at[r])]

    def xb_copy():
        return [pltpu.make_async_copy(bx, xbuf.at[1], xsem.at[NX])]

    def w_copy(k, g, sem, rows=slice(None)):
        src = (awq, bwq, awo_t, bwo_t)[k]
        return [pltpu.make_async_copy(src.at[rows, pl.ds(_mult(g, GW), GW)], wbuf.at[k * NG + g, rows], sem)]

    def wq_copy(p, g):
        return w_copy(p, g, qsem.at[(p * NG + g - 1) // QPN])

    def wo_copy(p, g, rows=slice(None)):
        return w_copy(2 + p, g, wsem.at[p * NG + g], rows)

    def b_slot(g):
        return (NG + 2 * g) & (RING - 1)

    def kv_copy(p, bs, src, dst, s, rows=slice(None)):
        return [pltpu.make_async_copy(cache.at[bs, src, rows], kvbuf.at[which, bs, dst, rows], kvsem.at[s])
                for which, cache in enumerate(((ak, av), (bk, bv))[p])]

    def kv_total(bs, dst, s):
        part = kvbuf.at[:, bs, dst]
        return [pltpu.make_async_copy(part, part, kvsem.at[s])]

    def group_wait(p, g):
        _wait(kv_total(slice(None), pl.ds(b_slot(g) if p else g, p + 1), p * NG + g) + wo_copy(p, g))

    def tail_sem(g, n):
        return NG + g if n == 0 else 2 * NG + (g - NG + 2) * (NCUT - 1) + n - 1

    def out_copy(t0, t1, c0=0, c1=NTILE):
        part = (pl.ds(t0 * 128, (t1 - t0) * 128), pl.ds(c0 * 128, (c1 - c0) * 128))
        return [pltpu.make_async_copy(obuf.at[part], out.at[part], osem)]

    def trickle_wo_a(half, m):
        n = D // (4 * NTILE)
        _start(wo_copy(0, half >> 1, pl.ds(pl.multiple_of((half & 1) * (D // 2) + m * n, n), n)), TRICKLE)

    def trickle_wo_b(i, m):
        n = D // (2 * NTILE)
        piece = wo_copy(1, i & (NG - 1), pl.ds(m * n, n))
        pl.when(i < NG)(lambda: _start(piece, TRICKLE))

    def trickled_unit(i):
        units = [(g, b) for g, n in enumerate(TRICKLED) for b in range(n)]
        groups = sum((g - k // 2 + 1) << (2 * k) for k, (g, _) in enumerate(units))
        batches = sum(b << (2 * k) for k, (_, b) in enumerate(units))
        return ((groups >> (2 * i)) & 3) + (i >> 1) - 1, (batches >> (2 * i)) & 3

    def trickle_kv(unit, m, which):
        g, b = unit
        j, r = divmod(m, SK // KV_ROWS)
        copies = kv_copy(1, b, 2 * g + j, b_slot(g) + j, NG + g, pl.ds(r * KV_ROWS, KV_ROWS))
        _start(copies[which:which + 1], TRICKLE)

    def bulk_copy(g, b0, b1, s):
        b0 = max(b0, TRICKLED[g])
        return kv_copy(1, pl.ds(b0, b1 - b0), pl.ds(2 * g, 2), pl.ds(b_slot(g), 2), s)

    def qproj(i, r0, n, c0, nc):
        q = jnp.dot(xbuf[i // NG, pl.ds(r0, n)], wbuf[i, :, c0 * 128:(c0 + nc) * 128],
                    preferred_element_type=F32)
        q = (q * SCALE).astype(BF16)
        for c in range(nc):
            qo[i * 4 + c0 + c, pl.ds(r0, n), :] = q[:, c * 128:(c + 1) * 128]

    def load_qo(kt, n, rows):
        return jnp.concatenate([qo[kt + c, rows, :] for c in range(n)], axis=1)

    def scores(i, b, j, slot):
        q = load_qo(i * 4 + 2 * j, 2, pl.ds(b * SQ, SQ))
        return lax.dot_general(q, kvbuf[0, b, slot], NT, preferred_element_type=F32)

    def attend(i, b, j, slot, s):
        e = jnp.exp2(s - jnp.max(s, axis=-1, keepdims=True))
        l = jnp.sum(e, axis=-1, keepdims=True)
        inv = pl.reciprocal(l, approx=True)
        inv = inv * (2.0 - l * inv)
        o = (jnp.dot(e.astype(BF16), kvbuf[1, b, slot], preferred_element_type=F32) * inv).astype(BF16)
        for c in range(2):
            qo[i * 4 + 2 * j + c, pl.ds(b * SQ, SQ), :] = o[:, c * 128:(c + 1) * 128]

    def oproj(i, t, t_acc, host=None):
        o = load_qo(i * 4, 4, pl.ds(t * 128, 128))
        parts = 1 if host is None else 2
        for h in range(parts):
            rows = pl.ds(h * D // parts, D // parts)
            acc[i // NG, t_acc, rows] += lax.dot_general(wbuf[2 * NG + i, rows], o, NT, preferred_element_type=F32)
            if host is not None:
                trickle_wo_b(host, 2 * t + h)

    def finish(t, c0=0, c1=NTILE):
        for c in range(c0, c1):
            lo, hi = c * 128, (c + 1) * 128
            parts = ([acc[0, t, lo:min(hi, D), :]] if lo < D else []) + \
                    ([acc[1, t, max(lo, D) - D:hi - D, :]] if hi > D else [])
            obuf[t * 128:(t + 1) * 128, lo:hi] = jnp.concatenate(parts, axis=0).T.astype(BF16)

    def group(i, slots, first=False, last=None, host=None, late=()):
        done = []
        unit = trickled_unit(i) if last is None else None

        def flush(b):
            if done and b >= CUTS[-2]:
                copies = out_copy(done[0], done[-1] + 1)
                pl.when(last)(lambda: _start(copies))
                done.clear()

        for b in range(NB):
            if last is not None and b in CUTS:
                n = CUTS.index(b)
                _wait(kv_total(pl.ds(b, CUTS[n + 1] - b), pl.ds(slots[0], 2), tail_sem(i - NG, n)))
                flush(b)
            s = []
            for j in range(2):
                s.append(scores(i, b, j, slots[j]))
                if last is None:
                    trickle_kv(unit, 2 * b + j, 0)
            if b == 0 and first:
                oproj(jnp.maximum(i - 1, 0), NTILE - 1, jnp.where(i == 0, NTILE, NTILE - 1), host)
            elif b == 0:
                oproj(i - 1, NTILE - 1, NTILE - 1, host)
            elif b >= 2:
                oproj(i, b - 2, b - 2, host)
                if last is not None:
                    finish(b - 2)
                    done.append(b - 2)
                    flush(b)
            for j in range(2):
                attend(i, b, j, slots[j], s[j])
                if last is None:
                    trickle_kv(unit, 2 * b + j, 1)
                if late:
                    copy = late.pop(0)
                    pl.when(i == NG)(lambda: _start([copy]))

    first_wq = w_copy(0, 0, xsem.at[NX + 1])
    _start(xa_copy(0) + first_wq)

    def issue_wq_a(g, carry):
        pl.when(g == 0)(lambda: _start(sum((xa_copy(r) for r in range(1, NX)), [])))
        pl.when(g > 0)(lambda: _start(wq_copy(0, g)))
    lax.fori_loop(0, NG, issue_wq_a, None)
    _start(xb_copy())
    lax.fori_loop(0, NG, lambda g, c: _start(wq_copy(1, g)), None)
    _start(wo_copy(0, NG - 1, pl.ds(D // 2, D // 2)))
    lax.fori_loop(0, NG, lambda g, c: _start(kv_copy(0, slice(None), g, g, g)), None)
    for g in range(NG // 2):
        _start(bulk_copy(g, 0, NB, NG + g))
    acc[...] = jnp.zeros(acc.shape, F32)

    _wait(first_wq)
    for r in range(NX):
        _wait(xa_copy(r))
        qproj(0, XCUTS[r], XCUTS[r + 1] - XCUTS[r], 0, 4)

    def q_step(n, carry):
        pl.when(n == (NG - 1) // QPN)(lambda: _wait(xb_copy()))
        chunks = wbuf.at[pl.ds(1 + n * QPN, QPN)]
        pltpu.make_async_copy(chunks, chunks, qsem.at[n]).wait()
        for d in range(QPN):
            i = 1 + n * QPN + d
            for m in range(NTILE):
                for j in range(2):
                    qproj(i, m * 128, 128, 2 * j, 2)
                    trickle_wo_a(i - 1, 2 * m + j)
    lax.fori_loop(0, NQSTEP, q_step, None)

    def pair_step(n, carry):
        @pl.when(2 * n < NG)
        def _():
            group_wait(0, 2 * n)
            group_wait(0, 2 * n + 1)

        @pl.when(2 * n >= NG)
        def _():
            group_wait(1, 2 * n - NG)
            group_wait(1, 2 * n + 1 - NG)
        late = sum((bulk_copy(g, 0, NB, NG + g) for g in range(NG // 2, NG - 2)), [])
        late += sum((bulk_copy(g, CUTS[k], CUTS[k + 1], tail_sem(g, k))
                     for g in (NG - 2, NG - 1) for k in range(NCUT)), [])
        for i, first in ((2 * n, True), (2 * n + 1, False)):
            group(i, [jnp.where(i < NG, i, b_slot(i - NG) + j) for j in range(2)], first, host=i, late=late)
    lax.fori_loop(0, NPAIR, pair_step, None)

    def single_step(g, carry):
        group_wait(1, g)
        group(NG + g, [b_slot(g), b_slot(g) + 1])
    lax.fori_loop(2 * NPAIR - NG, NG - 2, single_step, None)

    def tail_step(g, carry):
        _wait(wo_copy(1, g))
        group(NG + g, [b_slot(g), b_slot(g) + 1], last=g == NG - 1)
    lax.fori_loop(NG - 2, NG, tail_step, None)

    t = NTILE - 1
    finish(t, 0, 3)
    _start(out_copy(t, NTILE, 0, 3))
    oproj(2 * NG - 1, t, t)
    finish(t, 3, NTILE)
    _start(out_copy(t, NTILE, 3, NTILE), TRICKLE)
    pltpu.make_async_copy(obuf, out, osem).wait()


@jax.jit
def pallas_concat_heads__gqa_block_cached__mha_block_cached__near_ridge_kernel(
    A_x: jax.Array,
    A_k_cache: jax.Array,
    A_v_cache: jax.Array,
    A_wq: jax.Array,
    A_wo: jax.Array,
    B_x: jax.Array,
    B_k_cache: jax.Array,
    B_v_cache: jax.Array,
    B_wq: jax.Array,
    B_wo: jax.Array,
):
    hbm = pl.BlockSpec(memory_space=pl.ANY)
    out = pl.pallas_call(
        _body,
        out_shape=jax.ShapeDtypeStruct((T, 2 * D), BF16),
        in_specs=[hbm] * 10,
        out_specs=hbm,
        scratch_shapes=[
            pltpu.VMEM((2, T, D), BF16),
            pltpu.VMEM((4 * NG, D, GW), BF16),
            pltpu.VMEM((2, NB, RING, SK, DH), BF16),
            pltpu.VMEM((8 * NG, T, 128), BF16),
            pltpu.VMEM((2, NTILE + 1, D, 128), F32),
            pltpu.VMEM((T, 2 * D), BF16),
            pltpu.SemaphoreType.DMA((NX + 2,)),
            pltpu.SemaphoreType.DMA((NQSTEP,)),
            pltpu.SemaphoreType.DMA((2 * NG,)),
            pltpu.SemaphoreType.DMA((2 * NG + 2 * (NCUT - 1),)),
            pltpu.SemaphoreType.DMA(()),
        ],
        compiler_params=pltpu.CompilerParams(vmem_limit_bytes=120 * 2**20, disable_semaphore_checks=True),
    )(A_x.reshape(T, D), A_k_cache, A_v_cache, A_wq, A_wo.T,
      B_x.reshape(T, D), B_k_cache, B_v_cache, B_wq, B_wo.T)
    return out.reshape(NB, SQ, 2 * D)
```
